```python
import os as _os
_os.environ.setdefault("JAX_PLATFORMS", "cpu")
import jax
import jax.numpy as jnp

def _softmax(x, axis=-1):
    return jax.nn.softmax(x, axis=axis)
def _gelu(x):
    return jax.nn.gelu(x, approximate=True)
def _silu(x):
    return jax.nn.silu(x)
def _sigmoid(x):
    return jax.nn.sigmoid(x)
def _layernorm(x, axis=-1, eps=1e-5):
    m = jnp.mean(x, axis=axis, keepdims=True)
    v = jnp.var(x, axis=axis, keepdims=True)
    return (x - m) / jnp.sqrt(v + eps)
def _scatter_add(tgt, idx, src, axis=0):
    return tgt.at[idx].add(src)
def _segment_sum(src, seg, n):
    return jax.ops.segment_sum(src, seg, n)
class _Rng:
    def __init__(self, key):
        self._k = key
    def _next(self):
        self._k, sub = jax.random.split(self._k)
        return sub
    def normal(self, shape):
        return jax.random.normal(self._next(), shape, dtype=jnp.bfloat16)
    def randint(self, lo, hi, shape):
        return jax.random.randint(self._next(), shape, lo, hi, dtype=jnp.int32)
    def uniform(self, shape, lo=0.0, hi=1.0):
        return jax.random.uniform(self._next(), shape, jnp.bfloat16, lo, hi)
    def permutation(self, n):
        return jax.random.permutation(self._next(), n)


kernel_name = 'standalone__dense_activation_silu__prompt'

def setup_inputs():
    _rng = _Rng(jax.random.key(int.from_bytes(__import__("os").urandom(4), "little")))
    _w = (lambda a: (lambda t: t.astype(jnp.bfloat16) if jnp.issubdtype(t.dtype, jnp.floating) else t)(jnp.asarray(a)))
    B, S, D, F = 1, 2048, 448, 1792
    return {
        "x": _w((lambda *s: _rng.normal(s) * 0.05)(B, S, D)),
        "w1": _w((lambda *s: _rng.normal(s) * 0.05)(D, F) * (D ** -0.5)),
        "w2": _w((lambda *s: _rng.normal(s) * 0.05)(F, D) * (F ** -0.5)),
    }

def reference(x, w1, w2):
    h = jnp.einsum("bsd,df->bsf", x, w1)
    h = _silu(h)
    out = jnp.einsum("bsf,fd->bsd", h, w2)
    return out
```

```python
import jax
import jax.numpy as jnp
import jax.experimental.pallas as pl
import jax.experimental.pallas.tpu as pltpu


@jax.jit
def pallas_standalone__dense_activation_silu__prompt_kernel(
    x: jax.Array,
    w1: jax.Array,
    w2: jax.Array,
):
    B, S, D = x.shape
    F = w1.shape[1]
    M = B * S
    x2 = x.reshape(M, D)
    tm = 512

    def kernel_function(x_ref, w1_ref, w2_ref, o_ref):
        h = jnp.dot(x_ref[...], w1_ref[...], preferred_element_type=jnp.float32)
        h = h * jax.nn.sigmoid(h)
        o = jnp.dot(h.astype(jnp.bfloat16), w2_ref[...], preferred_element_type=jnp.float32)
        o_ref[...] = o.astype(o_ref.dtype)

    out = pl.pallas_call(
        kernel_function,
        grid=(M // tm,),
        in_specs=[
            pl.BlockSpec((tm, D), lambda i: (i, 0)),
            pl.BlockSpec((D, F), lambda i: (0, 0)),
            pl.BlockSpec((F, D), lambda i: (0, 0)),
        ],
        out_specs=pl.BlockSpec((tm, D), lambda i: (i, 0)),
        out_shape=jax.ShapeDtypeStruct((M, D), x.dtype),
        compiler_params=pltpu.CompilerParams(
            dimension_semantics=("arbitrary",),
            vmem_limit_bytes=64 * 1024 * 1024,
        ),
    )(x2, w1, w2)
    return out.reshape(B, S, D)
```

```python
import jax
import jax.numpy as jnp
import jax.experimental.pallas as pl
import jax.experimental.pallas.tpu as pltpu

BL = 128

_STAGES = ((2, 2), (4, 3), (6, 6), (14, 13))
_TILES = (4, 4, 4, 2, 1, 1)


def _silu(h):
    return h * pl.reciprocal(1.0 + jnp.exp(-h), approx=True)


def _cat(parts, axis):
    return parts[0] if len(parts) == 1 else jnp.concatenate(parts, axis=axis)


@jax.jit
def pallas_standalone__dense_activation_silu__prompt_kernel(
    x: jax.Array,
    w1: jax.Array,
    w2: jax.Array,
):
    B, S, D = x.shape
    F = w1.shape[1]
    M = B * S
    NS, NF = M // BL, F // BL
    assert M % BL == 0 and F % BL == 0 and sum(_TILES) == NS
    xT = x.reshape(M, D).T
    w2T = w2.T

    def kernel_function(xT_ref, w1_ref, w2T_ref, o_ref, xb, w1b, w2b, ob, sem):
        nsem = [0]

        def mk(src, dst, b0, b1):
            sl = pl.ds(b0 * BL, (b1 - b0) * BL)
            c = pltpu.make_async_copy(src.at[:, sl], dst.at[:, sl], sem.at[nsem[0]])
            nsem[0] += 1
            return c

        full = list(_STAGES) + [(NS, NF)]
        st_cps = []
        pa, pb = 0, 0
        for k, (a, b) in enumerate(full):
            cx = mk(xT_ref, xb, pa, a) if a > pa else None
            ca = mk(w1_ref, w1b, pb, b) if b > pb else None
            if k == len(full) - 1:
                lst = [ca, mk(w2T_ref, w2b, 0, NF), cx]
            else:
                lst = [ca, cx]
            st_cps.append([c for c in lst if c is not None])
            pa, pb = a, b
        for lst in st_cps:
            for c in lst:
                c.start()

        tr = {}
        g = {}

        def transpose(b0, b1):
            v = w1b[:, pl.ds(b0 * BL, (b1 - b0) * BL)].T
            for b in range(b0, b1):
                tr[b] = v[(b - b0) * BL:(b - b0 + 1) * BL, :]

        def mm1(s0, s1, f0, f1):
            if s1 <= s0 or f1 <= f0:
                return
            lhs = _cat([tr[b] for b in range(f0, f1)], 0)
            h = jnp.dot(lhs, xb[:, pl.ds(s0 * BL, (s1 - s0) * BL)],
                        preferred_element_type=jnp.float32)
            gg = _silu(h).astype(jnp.bfloat16)
            for s in range(s0, s1):
                for f in range(f0, f1):
                    g[(s, f)] = gg[(f - f0) * BL:(f - f0 + 1) * BL,
                                   (s - s0) * BL:(s - s0 + 1) * BL]

        def mm2(s0, s1):
            gg = _cat([_cat([g[(s, f)] for s in range(s0, s1)], 1) for f in range(NF)], 0)
            p = jnp.dot(w2b[...], gg, preferred_element_type=jnp.float32)
            ob[:, pl.ds(s0 * BL, (s1 - s0) * BL)] = p.astype(ob.dtype)

        pa, pb = 0, 0
        for k, (a, b) in enumerate(_STAGES):
            if k == 0:
                st_cps[0][0].wait()
                transpose(0, b)
                st_cps[0][1].wait()
                mm1(0, a, 0, b)
            else:
                for c in st_cps[k]:
                    c.wait()
                mm1(pa, a, 0, pb)
                if b > pb:
                    transpose(pb, b)
                mm1(0, a, pb, b)
            pa, pb = a, b
        for c in st_cps[-1]:
            c.wait()
        if pb < NF:
            transpose(pb, NF)
        ocs = []
        s0 = 0
        for t in _TILES:
            s1 = s0 + t
            mm1(max(s0, pa), s1, 0, NF)
            mm1(s0, min(s1, pa), pb, NF)
            mm2(s0, s1)
            oc = mk(ob, o_ref, s0, s1)
            oc.start()
            ocs.append(oc)
            s0 = s1
        for oc in ocs:
            oc.wait()

    outT = pl.pallas_call(
        kernel_function,
        in_specs=[pl.BlockSpec(memory_space=pl.ANY)] * 3,
        out_specs=pl.BlockSpec(memory_space=pl.ANY),
        out_shape=jax.ShapeDtypeStruct((D, M), x.dtype),
        scratch_shapes=[
            pltpu.VMEM((D, M), x.dtype),
            pltpu.VMEM((D, F), w1.dtype),
            pltpu.VMEM((D, F), w2.dtype),
            pltpu.VMEM((D, M), x.dtype),
            pltpu.SemaphoreType.DMA((2 * len(_STAGES) + 3 + len(_TILES),)),
        ],
        compiler_params=pltpu.CompilerParams(
            vmem_limit_bytes=100 * 1024 * 1024,
            disable_semaphore_checks=True,
        ),
    )(xT, w1, w2T)
    return outT.T.reshape(B, S, D)
```

```python
import jax
import jax.numpy as jnp
import jax.experimental.pallas as pl
import jax.experimental.pallas.tpu as pltpu

BL = 128
LOG2E = 1.4426950408889634


def _silu(h):
    return h * pl.reciprocal(1.0 + jnp.exp2(h * (-LOG2E)), approx=True)


def _cat(parts, axis):
    return parts[0] if len(parts) == 1 else jnp.concatenate(parts, axis=axis)


def _compiler_params():
    vmem = 100 * 1024 * 1024
    try:
        return pltpu.CompilerParams(vmem_limit_bytes=vmem, disable_semaphore_checks=True)
    except TypeError:
        return pltpu.CompilerParams(vmem_limit_bytes=vmem)


def _plan(NS, NF, D):
    b0, a1, b1, a2, b2, a4 = 2, 8, 7, 8, 10, 12
    whole = ((0, D),)
    tail_rows = ((0, 224), (224, 336), (336, 400), (400, D))
    p = [
        ('dma', 0, 'A', 3, 4, 0, b0),
        ('dma', 1, 'X', 3, 4, 0, a1), ('dma', 11, 'A', 3, 4, b0, b1),
        ('dma', 2, 'X', 3, 4, a1, NS), ('dma', 3, 'A', 3, 4, b1, NF),
        ('dma', 4, 'A', 0, 1, 0, b2), ('dma', 5, 'X', 0, 1, 0, a2),
        ('dma', 6, 'X', 0, 1, a2, NS), ('dma', 7, 'A', 0, 1, b2, NF),
        ('dma', 8, 'A', 1, 3, 0, NF), ('dma', 9, 'X', 1, 3, 0, NS),
        ('dma', 10, 'B', 0, 4, 0, NF),
        ('wait', 0), ('T', 3, 4, 0, b0),
        ('wait', 1, 11),
        ('mm', 3, 4, 0, a1, 0, b0), ('T', 3, 4, b0, b1), ('mm', 3, 4, 0, a1, b0, b1),
        ('wait', 2, 3, 4, 5),
        ('mm', 3, 4, a1, NS, 0, b1), ('T', 3, 4, b1, NF), ('mm', 3, 4, 0, NS, b1, NF),
        ('T', 0, 1, 0, b2), ('mm', 0, 1, 0, a2, 0, b2),
        ('wait', 6, 7, 8, 9, 10),
        ('mm', 0, 1, a2, a4, 0, b2),
        ('T', 0, 1, b2, NF), ('T', 1, 3, 0, NF),
        ('mm', 0, 3, a4, NS, 0, NF), ('out', a4, NS, whole),
    ]
    for s0 in range(0, a4, 4):
        s1 = s0 + 4
        p += [('mm', 1, 3, s0, s1, 0, b2), ('mm', 0, 3, s0, s1, b2, NF)]
        if s1 < a4:
            p += [('out', s0, s1, whole)]
        else:
            p += [('out', s0, s1 - 1, whole), ('out', s1 - 1, s1, tail_rows)]
    return p


@jax.jit
def pallas_standalone__dense_activation_silu__prompt_kernel(
    x: jax.Array,
    w1: jax.Array,
    w2: jax.Array,
):
    B, S, D = x.shape
    F = w1.shape[1]
    M = B * S
    assert (M, D, F) == (2048, 448, 1792), "schedule is tuned for these shapes"
    NS, NF = M // BL, F // BL
    KR = ((0, 128), (128, 256), (256, 384), (384, D))
    plan = _plan(NS, NF, D)
    n_sems = sum(1 if op[0] == 'dma' else len(op[3]) if op[0] == 'out' else 0 for op in plan)

    xT = x.reshape(M, D).T
    w2T = w2.T

    def kernel_function(xT_hbm, w1_hbm, w2T_hbm, o_hbm, xb, w1b, w2b, ob, sem):
        n_used = [0]

        def copy(src, dst, r0, r1, b0, b1):
            rows = pl.ds(r0, r1 - r0)
            cols = pl.ds(b0 * BL, (b1 - b0) * BL)
            c = pltpu.make_async_copy(src.at[rows, cols], dst.at[rows, cols], sem.at[n_used[0]])
            n_used[0] += 1
            c.start()
            return c

        arrays = {'X': (xT_hbm, xb), 'A': (w1_hbm, w1b), 'B': (w2T_hbm, w2b)}
        in_flight = {}
        out_copies = []
        w1T = {}
        part = {}
        n_done = {}
        gT = {}

        for op in plan:
            if op[0] == 'dma':
                _, i, name, k0, k1, b0, b1 = op
                src, dst = arrays[name]
                in_flight[i] = copy(src, dst, KR[k0][0], KR[k1 - 1][1], b0, b1)
            elif op[0] == 'wait':
                for i in op[1:]:
                    in_flight.pop(i).wait()
            elif op[0] == 'T':
                _, k0, k1, f0, f1 = op
                r0, r1 = KR[k0][0], KR[k1 - 1][1]
                v = w1b[pl.ds(r0, r1 - r0), pl.ds(f0 * BL, (f1 - f0) * BL)].T
                for f in range(f0, f1):
                    for k in range(k0, k1):
                        w1T[(k, f)] = v[(f - f0) * BL:(f - f0 + 1) * BL,
                                        KR[k][0] - r0:KR[k][1] - r0]
            elif op[0] == 'mm':
                _, k0, k1, s0, s1, f0, f1 = op
                r0, r1 = KR[k0][0], KR[k1 - 1][1]
                units = [(s, f) for f in range(f0, f1) for s in range(s0, s1)]
                lhs = _cat([_cat([w1T[(k, f)] for k in range(k0, k1)], 1)
                            for f in range(f0, f1)], 0)
                h = jnp.dot(lhs, xb[pl.ds(r0, r1 - r0), pl.ds(s0 * BL, (s1 - s0) * BL)],
                            preferred_element_type=jnp.float32)
                if units[0] in part:
                    h = h + _cat([_cat([part.pop((s, f)) for s in range(s0, s1)], 1)
                                  for f in range(f0, f1)], 0)
                for u in units:
                    n_done[u] = n_done.get(u, 0) + (k1 - k0)
                    assert n_done[u] == n_done[units[0]] and u not in part
                if n_done[units[0]] == len(KR):
                    h, dst = _silu(h).astype(jnp.bfloat16), gT
                else:
                    dst = part
                for (s, f) in units:
                    dst[(s, f)] = h[(f - f0) * BL:(f - f0 + 1) * BL,
                                    (s - s0) * BL:(s - s0 + 1) * BL]
            else:
                _, s0, s1, row_splits = op
                g = _cat([_cat([gT.pop((s, f)) for s in range(s0, s1)], 1)
                          for f in range(NF)], 0)
                o = jnp.dot(w2b[...], g, preferred_element_type=jnp.float32).astype(ob.dtype)
                for (r0, r1) in row_splits:
                    ob[pl.ds(r0, r1 - r0), pl.ds(s0 * BL, (s1 - s0) * BL)] = o[r0:r1]
                    out_copies.append(copy(ob, o_hbm, r0, r1, s0, s1))
        assert not in_flight and not part and not gT and n_used[0] == n_sems
        for c in out_copies:
            c.wait()

    outT = pl.pallas_call(
        kernel_function,
        in_specs=[pl.BlockSpec(memory_space=pl.ANY)] * 3,
        out_specs=pl.BlockSpec(memory_space=pl.ANY),
        out_shape=jax.ShapeDtypeStruct((D, M), x.dtype),
        scratch_shapes=[
            pltpu.VMEM((D, M), x.dtype),
            pltpu.VMEM((D, F), w1.dtype),
            pltpu.VMEM((D, F), w2.dtype),
            pltpu.VMEM((D, M), x.dtype),
            pltpu.SemaphoreType.DMA((n_sems,)),
        ],
        compiler_params=_compiler_params(),
    )(xT, w1, w2T)
    return outT.T.reshape(B, S, D)
```
